```python
import jax
import jax.numpy as jnp

def _softmax(x, axis=-1):
    return jax.nn.softmax(x, axis=axis)
def _gelu(x):
    return jax.nn.gelu(x, approximate=True)
def _silu(x):
    return jax.nn.silu(x)
def _sigmoid(x):
    return jax.nn.sigmoid(x)
def _layernorm(x, axis=-1, eps=1e-5):
    m = jnp.mean(x, axis=axis, keepdims=True)
    v = jnp.var(x, axis=axis, keepdims=True)
    return (x - m) / jnp.sqrt(v + eps)
def _scatter_add(tgt, idx, src, axis=0):
    return tgt.at[idx].add(src)
def _segment_sum(src, seg, n):
    return jax.ops.segment_sum(src, seg, n)
class _Rng:
    def __init__(self, key):
        self._k = key
    def _next(self):
        self._k, sub = jax.random.split(self._k)
        return sub
    def normal(self, shape):
        return jax.random.normal(self._next(), shape, dtype=jnp.bfloat16)
    def randint(self, lo, hi, shape):
        return jax.random.randint(self._next(), shape, lo, hi, dtype=jnp.int32)
    def uniform(self, shape, lo=0.0, hi=1.0):
        return jax.random.uniform(self._next(), shape, jnp.bfloat16, lo, hi)
    def permutation(self, n):
        return jax.random.permutation(self._next(), n)


kernel_name = 'standalone__structured_sparse_n_m__ragged'

def setup_inputs():
    _rng = _Rng(jax.random.key(int.from_bytes(__import__("os").urandom(4), "little")))
    _w = (lambda a: (lambda t: t.astype(jnp.bfloat16) if jnp.issubdtype(t.dtype, jnp.floating) else t)(jnp.asarray(a)))
    B, S, D = 16, 4096, 576
    assert D % 4 == 0, "d_model must be divisible by M=4 for 2:4 sparsity"
    return {
        "x": _w((lambda *s: _rng.normal(s) * 0.05)(B, S, D)),
        "w": _w((lambda *s: _rng.normal(s) * 0.05)(D, D)),
        "b": _w((lambda *s: _rng.normal(s) * 0.05)(D)),
    }

def reference(x, w, b):
    B, S, D = x.shape
    N, M = 2, 4
    G = D // M
    wg = w.reshape(G, M, D)
    mag = jnp.abs(wg)
    order = jnp.argsort(mag, 1)
    thr = jnp.take_along_axis(mag, order[:, M - N:M - N + 1, :], 1)
    mask = (lambda x, dt: x.astype(dt))(mag >= thr, w.dtype)
    wp = (wg * mask).reshape(D, D)
    return jnp.einsum("bsd,df->bsf", x, wp) + b
```

```python
import jax
import jax.numpy as jnp
import jax.experimental.pallas as pl
import jax.experimental.pallas.tpu as pltpu


def _prune(w):
    D = w.shape[0]
    wf = w.astype(jnp.float32)
    mag = jnp.abs(wf)
    row = jax.lax.broadcasted_iota(jnp.int32, wf.shape, 0) % 4
    cnt = jnp.zeros(wf.shape, jnp.float32)
    for sh in (1, 2, 3):
        up = pltpu.roll(mag, sh, 0)
        dn = pltpu.roll(mag, D - sh, 0)
        cnt += jnp.where((row >= sh) & (up > mag), 1.0, 0.0)
        cnt += jnp.where((row + sh <= 3) & (dn > mag), 1.0, 0.0)
    return jnp.where(cnt <= 1.0, wf, 0.0)


@jax.jit
def pallas_standalone__structured_sparse_n_m__ragged_kernel(
    x: jax.Array,
    w: jax.Array,
    b: jax.Array,
):
    B, S, D = x.shape
    ts = 2048

    def kernel_function(x_ref, w_ref, b_ref, o_ref, wt_ref):
        @pl.when((pl.program_id(0) == 0) & (pl.program_id(1) == 0))
        def _():
            wt_ref[...] = _prune(w_ref[...]).T.astype(jnp.bfloat16)

        acc = jnp.dot(wt_ref[...], x_ref[...], preferred_element_type=jnp.float32)
        o_ref[...] = (acc + b_ref[...]).astype(o_ref.dtype)

    xt = jnp.transpose(x, (0, 2, 1))
    b2 = b.astype(jnp.float32).reshape(D, 1)
    ot = pl.pallas_call(
        kernel_function,
        grid=(B, S // ts),
        in_specs=[
            pl.BlockSpec((None, D, ts), lambda i, j: (i, 0, j)),
            pl.BlockSpec((D, D), lambda i, j: (0, 0)),
            pl.BlockSpec((D, 1), lambda i, j: (0, 0)),
        ],
        out_specs=pl.BlockSpec((None, D, ts), lambda i, j: (i, 0, j)),
        out_shape=jax.ShapeDtypeStruct((B, D, S), x.dtype),
        scratch_shapes=[pltpu.VMEM((D, D), jnp.bfloat16)],
        compiler_params=pltpu.CompilerParams(
            dimension_semantics=("arbitrary", "arbitrary"),
            vmem_limit_bytes=100 * 1024 * 1024,
        ),
    )(xt, w, b2)
    return jnp.transpose(ot, (0, 2, 1))
```

```python
import jax
import jax.numpy as jnp
import jax.experimental.pallas as pl
import jax.experimental.pallas.tpu as pltpu
from jax import lax

_LANES = 128
_NX = 3
_NO = 3
_NH = 4
_NCH = 16


def _prune_packed(w):
    f32, i32 = jnp.float32, jnp.int32
    D = w.shape[0]
    v = pltpu.bitcast(w, i32).reshape(D // 16, 8, D)
    a0 = pltpu.bitcast((v & 0x7FFF) << 16, f32)
    a1 = pltpu.bitcast(v & 0x7FFF0000, f32)
    hi = jnp.maximum(a0, a1)
    lo = jnp.minimum(a0, a1)
    even = (lax.broadcasted_iota(i32, v.shape, 1) & 1) == 0
    hi2 = jnp.where(even, pltpu.roll(hi, 7, 1), pltpu.roll(hi, 1, 1))
    lo2 = jnp.where(even, pltpu.roll(lo, 7, 1), pltpu.roll(lo, 1, 1))
    thr = jnp.maximum(jnp.minimum(hi, hi2), jnp.maximum(lo, lo2))
    k0 = jnp.where(a0 < thr, 0, 0xFFFF)
    k1 = jnp.where(a1 < thr, 0, -65536)
    return pltpu.bitcast((v & (k0 | k1)).reshape(D // 2, D), jnp.bfloat16)


@jax.jit
def pallas_standalone__structured_sparse_n_m__ragged_kernel(
    x: jax.Array,
    w: jax.Array,
    b: jax.Array,
):
    f32, bf16, i32 = jnp.float32, jnp.bfloat16, jnp.int32
    B, S, D = x.shape
    KH = (D // (2 * _LANES)) * _LANES
    KR = D - 2 * KH
    H = D // 2
    PAIR = 2 * _LANES
    assert x.dtype == bf16 and w.dtype == bf16 and b.dtype == bf16
    assert KH > 0 and KR + 16 <= _LANES and D % 32 == 0 and B >= _NX
    hw = S // _NH
    cw = S // _NCH
    assert hw % PAIR == 0 and cw % PAIR == 0

    def kernel_function(x_hbm, w_hbm, b_ref, o_hbm, xb, ob, wv, a_ref, t_ref,
                        hsem, rsem, wsem, sem):
        def dot(p, q):
            return jnp.dot(p, q, preferred_element_type=f32)

        def mo(v, n):
            return v if isinstance(v, int) else pl.multiple_of(v, n)

        def rd(g):
            return pltpu.make_async_copy(x_hbm.at[g], xb.at[g % _NX], rsem.at[g % _NX])

        def head_rd(j):
            cols = pl.ds(mo(j * hw, hw), hw)
            return pltpu.make_async_copy(x_hbm.at[0, :, cols], xb.at[0, :, cols], hsem.at[j])

        def wr_start(g, slot, c0, n):
            cols = pl.ds(c0, n)
            pltpu.make_async_copy(ob.at[slot, :, cols], o_hbm.at[g, :, cols], wsem.at[slot]).start()

        def wr_wait(g):
            pltpu.make_async_copy(ob.at[g % _NO], o_hbm.at[g], wsem.at[g % _NO]).wait()

        wcp = pltpu.make_async_copy(w_hbm, wv, sem)
        wcp.start()
        head_rd(0).start()
        wcp.wait()
        head_rd(1).start()

        wp = _prune_packed(wv[...])
        first = lax.broadcasted_iota(i32, (16, D), 0) == 0
        brow = jnp.where(first, jnp.broadcast_to(b_ref[...].astype(f32)[None, :], (16, D)), 0.0)
        zpad = jnp.zeros((_LANES - KR - 16, D), bf16)
        wt = jnp.concatenate([wp, brow.astype(bf16), zpad], axis=0).T
        A11, A12 = wt[:H, :KH], wt[:H, KH:2 * KH]
        A21, A22 = wt[H:, :KH], wt[H:, KH:2 * KH]
        g11, g12, g21, g22 = (v.astype(f32) for v in (A11, A12, A21, A22))
        for i, val in enumerate((
                (g11 + g22).astype(bf16), (g21 + g22).astype(bf16), A11, A22,
                (g11 + g12).astype(bf16), (g21 - g11).astype(bf16), (g12 - g22).astype(bf16))):
            a_ref[i] = pltpu.bitcast(val, i32)
        t_ref[...] = pltpu.bitcast(wt[:, 2 * KH:], i32)

        def A(i):
            return pltpu.bitcast(a_ref[i], bf16)

        def compute_pair(x_ref, o_ref):
            P, Q = pl.ds(0, _LANES), pl.ds(_LANES, _LANES)
            B11, B12 = x_ref[0:KH, P], x_ref[0:KH, Q]
            B21, B22 = x_ref[KH:2 * KH, P], x_ref[KH:2 * KH, Q]
            f11, f12, f21, f22 = (v.astype(f32) for v in (B11, B12, B21, B22))
            M1 = dot(A(0), (f11 + f22).astype(bf16))
            M2 = dot(A(1), B11)
            M3 = dot(A(2), (f12 - f22).astype(bf16))
            M4 = dot(A(3), (f21 - f11).astype(bf16))
            M5 = dot(A(4), B22)
            M6 = dot(A(5), (f11 + f12).astype(bf16))
            M7 = dot(A(6), (f21 + f22).astype(bf16))
            ones = jnp.where(lax.broadcasted_iota(i32, (_LANES - KR, _LANES), 0) == 0, 1.0, 0.0)
            ones = ones.astype(bf16)
            T = pltpu.bitcast(t_ref[...], bf16)
            TP = dot(T, jnp.concatenate([x_ref[2 * KH:, P], ones], axis=0))
            TQ = dot(T, jnp.concatenate([x_ref[2 * KH:, Q], ones], axis=0))
            o_ref[0:H, P] = (M1 + M4 - M5 + M7 + TP[:H]).astype(bf16)
            o_ref[0:H, Q] = (M3 + M5 + TQ[:H]).astype(bf16)
            o_ref[H:, P] = (M2 + M4 + TP[H:]).astype(bf16)
            o_ref[H:, Q] = (M1 - M2 + M3 + M6 + TQ[H:]).astype(bf16)

        def compute_cols(xs, os_, c0, n):
            for c in range(n // PAIR):
                cols = pl.ds(mo(c0 + c * PAIR, PAIR), PAIR)
                compute_pair(xb.at[xs, :, cols], ob.at[os_, :, cols])

        def head(j, carry):
            head_rd(j).wait()

            @pl.when(j == 0)
            def _():
                for jj in range(2, _NH):
                    head_rd(jj).start()

            @pl.when(j == 1)
            def _():
                rd(1).start()

            @pl.when(j == _NH - 1)
            def _():
                rd(2).start()

            compute_cols(0, 0, j * hw, hw)
            return carry

        lax.fori_loop(0, _NH, head, None)
        wr_start(0, 0, 0, S)

        def body(g, carry):
            @pl.when(g >= _NO)
            def _():
                wr_wait(g - _NO)

            rd(g).wait()
            slot = g % _NO
            for j in range(_NCH):
                compute_cols(g % _NX, slot, j * cw, cw)
                if j == 0:
                    @pl.when(g + 2 < B)
                    def _():
                        rd(g + 2).start()
                wr_start(g, slot, j * cw, cw)
            return carry

        lax.fori_loop(1, B, body, None)
        for g in range(B - _NO, B):
            wr_wait(g)

    xt = jnp.transpose(x, (0, 2, 1))
    ot = pl.pallas_call(
        kernel_function,
        in_specs=[
            pl.BlockSpec(memory_space=pl.ANY),
            pl.BlockSpec(memory_space=pl.ANY),
            pl.BlockSpec(memory_space=pltpu.VMEM),
        ],
        out_specs=pl.BlockSpec(memory_space=pl.ANY),
        out_shape=jax.ShapeDtypeStruct((B, D, S), x.dtype),
        scratch_shapes=[
            pltpu.VMEM((_NX, D, S), bf16),
            pltpu.VMEM((_NO, D, S), bf16),
            pltpu.VMEM((D, D), bf16),
            pltpu.VMEM((7, H // 2, KH), i32),
            pltpu.VMEM((D // 2, _LANES), i32),
            pltpu.SemaphoreType.DMA((_NH,)),
            pltpu.SemaphoreType.DMA((_NX,)),
            pltpu.SemaphoreType.DMA((_NO,)),
            pltpu.SemaphoreType.DMA(()),
        ],
        compiler_params=pltpu.CompilerParams(
            vmem_limit_bytes=64 * 1024 * 1024,
            disable_bounds_checks=True,
        ),
    )(xt, w, b)
    return jnp.transpose(ot, (0, 2, 1))
```

```python
import jax
import jax.numpy as jnp
import jax.experimental.pallas as pl
import jax.experimental.pallas.tpu as pltpu
from jax import lax

_D = 576
_H = 288
_PAIR = 256
_NX = 4
_NO = 4
_NH = 4


def _prune_packed(w):
    f32, i32 = jnp.float32, jnp.int32
    R, C = w.shape
    v = pltpu.bitcast(w, i32).reshape(R // 16, 8, C)
    a0 = pltpu.bitcast((v & 0x7FFF) << 16, f32)
    a1 = pltpu.bitcast(v & 0x7FFF0000, f32)
    hi = jnp.maximum(a0, a1)
    lo = jnp.minimum(a0, a1)
    even = (lax.broadcasted_iota(i32, v.shape, 1) & 1) == 0
    hi2 = jnp.where(even, pltpu.roll(hi, 7, 1), pltpu.roll(hi, 1, 1))
    lo2 = jnp.where(even, pltpu.roll(lo, 7, 1), pltpu.roll(lo, 1, 1))
    thr = jnp.maximum(jnp.minimum(hi, hi2), jnp.maximum(lo, lo2))
    k0 = jnp.where(a0 < thr, 0, 0xFFFF)
    k1 = jnp.where(a1 < thr, 0, -65536)
    return pltpu.bitcast((v & (k0 | k1)).reshape(R // 2, C), jnp.bfloat16)


def _prepare_weights(w, l_ref, e_ref):
    f32, bf16, i32 = jnp.float32, jnp.bfloat16, jnp.int32
    wp = _prune_packed(w)
    g = jnp.concatenate([wp, wp[512:]], axis=0).T.astype(f32)
    low = lax.broadcasted_iota(i32, (_H, 128), 1) < 64

    def tile(r, c):
        return g[r * _H:(r + 1) * _H, c * 128:(c + 1) * 128]

    def mix(p, q):
        return jnp.where(low, p, q)

    def add(p, q):
        return p[0] + q[0], p[1] + q[1]

    def sub(p, q):
        return p[0] - q[0], p[1] - q[1]

    A11, A12 = (tile(0, 0), tile(0, 1)), (tile(0, 2), tile(0, 3))
    A21, A22 = (tile(1, 0), tile(1, 1)), (tile(1, 2), tile(1, 3))
    top, bot = tile(0, 4), tile(1, 4)
    s1, s2, s5 = add(A11, A22), add(A21, A22), add(A11, A12)
    s6, s7 = sub(A21, A11), sub(A12, A22)
    wide = ((s1[0], mix(s1[1], 0.0)),
            (s2[0], mix(s2[1], -s2[1])),
            (A11[0], mix(A11[1], -A22[1])),
            (A22[0], mix(A22[1], -A11[1])),
            (s5[0], mix(s5[1], -s5[1])),
            (s6[0], mix(s6[1], bot)),
            (s7[0], mix(s7[1], top)))
    for i, pq in enumerate(wide):
        l_ref[i] = pltpu.bitcast(jnp.concatenate(pq, axis=1).astype(bf16), i32)
    narrow = (mix(pltpu.roll(s1[1], 64, 1), 0.0), mix(top, s7[1]), mix(bot, s6[1]))
    for i, v in enumerate(narrow):
        e_ref[i] = pltpu.bitcast(v.astype(bf16), i32)


def _compute_pair(x_ref, o_ref, l_ref, e_ref, bias_ref):
    f32, bf16 = jnp.float32, jnp.bfloat16

    def L(i, t):
        return jnp.dot(pltpu.bitcast(l_ref[i], bf16), t, preferred_element_type=f32)

    def E(i, t):
        return jnp.dot(pltpu.bitcast(e_ref[i], bf16), t, preferred_element_type=f32)

    def cat(p, q):
        return jnp.concatenate([p, q], axis=0)

    P, Q = pl.ds(0, 128), pl.ds(128, 128)
    B11, B12 = x_ref[0:256, P], x_ref[0:256, Q]
    B21, B22 = x_ref[256:512, P], x_ref[256:512, Q]
    XP, XQ = x_ref[512:, P], x_ref[512:, Q]
    f11, f12, f21, f22 = (v.astype(f32) for v in (B11, B12, B21, B22))
    zero = jnp.zeros((64, 128), bf16)
    S6, S7 = (f11 + f12).astype(bf16), (f21 + f22).astype(bf16)
    M1 = L(0, cat((f11[:192] + f22[:192]).astype(bf16), zero))
    M2 = L(1, cat(B11[:192], B12[192:]))
    M3 = L(2, (f12 - f22).astype(bf16))
    M4 = L(3, (f21 - f11).astype(bf16))
    M5 = L(4, cat(B22[:192], B21[192:]))
    M6 = L(5, cat(S6[:192], XQ))
    M7 = L(6, cat(S7[:192], XP))
    N1 = E(0, cat((f12[192:] + f21[192:]).astype(bf16), zero))
    E2 = E(1, cat(XQ, S7[192:])) + bias_ref[:_H]
    E3 = E(2, cat(XP, S6[192:])) + bias_ref[_H:]
    o_ref[:_H, P] = (M1 + M4 - M5 + M7 + bias_ref[:_H]).astype(bf16)
    o_ref[:_H, Q] = (M3 + M5 + N1 + E2).astype(bf16)
    o_ref[_H:, P] = (M2 + M4 + N1 + E3).astype(bf16)
    o_ref[_H:, Q] = (M1 - M2 + M3 + M6 + bias_ref[_H:]).astype(bf16)


@jax.jit
def pallas_standalone__structured_sparse_n_m__ragged_kernel(
    x: jax.Array,
    w: jax.Array,
    b: jax.Array,
):
    f32, bf16, i32 = jnp.float32, jnp.bfloat16, jnp.int32
    B, S, D = x.shape
    assert D == _D and x.dtype == w.dtype == b.dtype == bf16
    assert B % 2 == 0 and B >= 6 and S % (_NH * _PAIR) == 0
    hw = S // _NH
    NP = S // _PAIR

    def kernel_function(x_hbm, w_hbm, b_ref, o_hbm, xb, ob, wv, l_ref, e_ref, bias_ref,
                        hsem, rsem, wsem, sem):
        def rd(g):
            return pltpu.make_async_copy(x_hbm.at[g], xb.at[g % _NX], rsem.at[g % _NX])

        def head_rd(j):
            cols = pl.ds(j * hw if isinstance(j, int) else pl.multiple_of(j * hw, hw), hw)
            return pltpu.make_async_copy(x_hbm.at[0, :, cols], xb.at[0, :, cols], hsem.at[j])

        def wr_start(g, pairs):
            for p in pairs:
                cols = pl.ds(p * _PAIR, _PAIR)
                pltpu.make_async_copy(
                    ob.at[g % _NO, :, cols], o_hbm.at[g, :, cols], wsem.at[g % _NO]).start()

        def wr_wait(g):
            pltpu.make_async_copy(ob.at[g % _NO], o_hbm.at[g], wsem.at[g % _NO]).wait()

        def pair(xs, os_, c0):
            cols = pl.ds(c0, _PAIR)
            _compute_pair(xb.at[xs, :, cols], ob.at[os_, :, cols], l_ref, e_ref, bias_ref)

        wcp = pltpu.make_async_copy(w_hbm, wv, sem)
        wcp.start()
        head_rd(0).start()
        bias_ref[...] = jnp.broadcast_to(b_ref[...].astype(f32)[None, :], (128, D)).T
        wcp.wait()
        head_rd(1).start()
        _prepare_weights(wv[...], l_ref, e_ref)

        def head(j, carry):
            head_rd(j).wait()

            @pl.when(j == 0)
            def _():
                for jj in range(2, _NH):
                    head_rd(jj).start()
                rd(1).start()

            @pl.when(j == _NH // 2)
            def _():
                rd(2).start()

            for c in range(hw // _PAIR):
                pair(0, 0, pl.multiple_of(j * hw + c * _PAIR, _PAIR))
            return carry

        lax.fori_loop(0, _NH, head, None)

        def body(g, carry):
            @pl.when(g >= _NO)
            def _():
                wr_wait(g - _NO)

            rd(g).wait()
            odd = g % 2 == 1
            for p in range(NP):
                pair(g % _NX, g % _NO, p * _PAIR)
                if p == 0:
                    for k in (2, 3):
                        @pl.when(odd & (g + k < B))
                        def _():
                            rd(g + k).start()

                    @pl.when(~odd & (g < B - 2))
                    def _():
                        wr_start(g - 2, range(NP))

                    @pl.when(~odd)
                    def _():
                        wr_start(g - 1, range(NP))

                if p == NP // 2 - 1:
                    @pl.when(g == B - 3)
                    def _():
                        wr_start(g - 1, range(NP))

                @pl.when(g >= B - 2)
                def _():
                    wr_start(g, [p])
            return carry

        lax.fori_loop(1, B, body, None)
        for g in range(B - _NO, B):
            wr_wait(g)

    xt = jnp.transpose(x, (0, 2, 1))
    ot = pl.pallas_call(
        kernel_function,
        in_specs=[
            pl.BlockSpec(memory_space=pl.ANY),
            pl.BlockSpec(memory_space=pl.ANY),
            pl.BlockSpec(memory_space=pltpu.VMEM),
        ],
        out_specs=pl.BlockSpec(memory_space=pl.ANY),
        out_shape=jax.ShapeDtypeStruct((B, D, S), x.dtype),
        scratch_shapes=[
            pltpu.VMEM((_NX, D, S), bf16),
            pltpu.VMEM((_NO, D, S), bf16),
            pltpu.VMEM((D, D), bf16),
            pltpu.VMEM((7, _H // 2, 256), i32),
            pltpu.VMEM((3, _H // 2, 128), i32),
            pltpu.VMEM((D, 128), f32),
            pltpu.SemaphoreType.DMA((_NH,)),
            pltpu.SemaphoreType.DMA((_NX,)),
            pltpu.SemaphoreType.DMA((_NO,)),
            pltpu.SemaphoreType.DMA(()),
        ],
        compiler_params=pltpu.CompilerParams(
            vmem_limit_bytes=64 * 1024 * 1024,
            disable_bounds_checks=True,
        ),
    )(xt, w, b)
    return jnp.transpose(ot, (0, 2, 1))
```

```python
import jax
import jax.numpy as jnp
import jax.experimental.pallas as pl
import jax.experimental.pallas.tpu as pltpu
from jax import lax

_D = 576
_H = 288
_PAIR = 256
_UNIT = 20
_PIECE = 4
_HEAD = ((2, 2), (4, 1), (8, 1))
_W_PIECES = ((512, 64), (0, 128), (256, 128), (128, 128), (384, 128))


def _prune_packed(w):
    f32, i32 = jnp.float32, jnp.int32
    R, C = w.shape
    v = pltpu.bitcast(w, i32).reshape(R // 16, 8, C)
    a0 = pltpu.bitcast((v & 0x7FFF) << 16, f32)
    a1 = pltpu.bitcast(v & 0x7FFF0000, f32)
    hi = jnp.maximum(a0, a1)
    lo = jnp.minimum(a0, a1)
    even = (lax.broadcasted_iota(i32, v.shape, 1) & 1) == 0
    hi2 = jnp.where(even, pltpu.roll(hi, 7, 1), pltpu.roll(hi, 1, 1))
    lo2 = jnp.where(even, pltpu.roll(lo, 7, 1), pltpu.roll(lo, 1, 1))
    thr = jnp.maximum(jnp.minimum(hi, hi2), jnp.maximum(lo, lo2))
    k0 = jnp.where(a0 < thr, 0, 0xFFFF)
    k1 = jnp.where(a1 < thr, 0, -65536)
    return pltpu.bitcast((v & (k0 | k1)).reshape(R // 2, C), jnp.bfloat16)


def _prepare_weights(wait, wv, l_ref, e_ref):
    f32, bf16, i32 = jnp.float32, jnp.bfloat16, jnp.int32
    h = _H // 2
    low = lax.broadcasted_iota(i32, (h, 128), 1) < 64

    def piece(i):
        wait(i)
        r0, n = _W_PIECES[i]
        wp = _prune_packed(wv[r0:r0 + n])
        if n == 64:
            wp = jnp.concatenate([wp, wp], axis=0)
        v = pltpu.bitcast(wp.T, i32)
        return v[:h], v[h:]

    def mix(p, q):
        return jnp.where(low, p, q)

    def neg(p):
        return p ^ jnp.int32(-0x7FFF8000)

    def up(p):
        return pltpu.bitcast(p, bf16).astype(f32)

    def down(p):
        return pltpu.bitcast(p.astype(bf16), i32)

    top, bot = piece(0)
    for t in range(2):
        a11, a21 = piece(1 + 2 * t)
        f11, f21 = up(a11), up(a21)
        s6 = down(f21 - f11)
        a12, a22 = piece(2 + 2 * t)
        f12, f22 = up(a12), up(a22)
        s1, s2, s5, s7 = down(f11 + f22), down(f21 + f22), down(f11 + f12), down(f12 - f22)
        if t == 0:
            tiles = (s1, s2, a11, a22, s5, s6, s7)
        else:
            tiles = (mix(s1, 0), mix(s2, neg(s2)), mix(a11, neg(a22)), mix(a22, neg(a11)),
                     mix(s5, neg(s5)), mix(s6, bot), mix(s7, top))
            e_ref[0] = mix(pltpu.roll(s1, 64, 1), 0)
            e_ref[1] = mix(top, s7)
            e_ref[2] = mix(bot, s6)
        for i, tile in enumerate(tiles):
            l_ref[i, :, t * 128:(t + 1) * 128] = tile


def _compute_pair(x_ref, o_ref, l_ref, e_ref, bias_ref):
    f32, bf16 = jnp.float32, jnp.bfloat16

    def L(i, t):
        return jnp.dot(pltpu.bitcast(l_ref[i], bf16), t, preferred_element_type=f32)

    def E(i, t):
        return jnp.dot(pltpu.bitcast(e_ref[i], bf16), t, preferred_element_type=f32)

    def cat(p, q):
        return jnp.concatenate([p, q], axis=0)

    P, Q = pl.ds(0, 128), pl.ds(128, 128)
    B11, B12 = x_ref[0:256, P], x_ref[0:256, Q]
    B21, B22 = x_ref[256:512, P], x_ref[256:512, Q]
    XP, XQ = x_ref[512:, P], x_ref[512:, Q]
    f11, f12, f21, f22 = (v.astype(f32) for v in (B11, B12, B21, B22))
    zero = jnp.zeros((64, 128), bf16)
    M5 = L(4, cat(B22[:192], B21[192:]))
    M2 = L(1, cat(B11[:192], B12[192:]))
    N1 = E(0, cat((f12[192:] + f21[192:]).astype(bf16), zero))
    M4 = L(3, (f21 - f11).astype(bf16))
    M3 = L(2, (f12 - f22).astype(bf16))
    M1 = L(0, cat((f11[:192] + f22[:192]).astype(bf16), zero))
    M6 = L(5, cat((f11[:192] + f12[:192]).astype(bf16), XQ))
    M7 = L(6, cat((f21[:192] + f22[:192]).astype(bf16), XP))
    E2 = E(1, cat(XQ, (f21[192:] + f22[192:]).astype(bf16)))
    E3 = E(2, cat(XP, (f11[192:] + f12[192:]).astype(bf16)))
    o_ref[:_H, P] = (M1 + M4 - M5 + M7 + bias_ref[:_H]).astype(bf16)
    o_ref[:_H, Q] = (M3 + M5 + N1 + E2 + bias_ref[:_H]).astype(bf16)
    o_ref[_H:, P] = (M2 + M4 + N1 + E3 + bias_ref[_H:]).astype(bf16)
    o_ref[_H:, Q] = (M1 - M2 + M3 + M6 + bias_ref[_H:]).astype(bf16)


@jax.jit
def pallas_standalone__structured_sparse_n_m__ragged_kernel(
    x: jax.Array,
    w: jax.Array,
    b: jax.Array,
):
    f32, bf16, i32 = jnp.float32, jnp.bfloat16, jnp.int32
    B, S, D = x.shape
    assert D == _D and x.dtype == w.dtype == b.dtype == bf16
    NP = S // _PAIR
    log_np = NP.bit_length() - 1
    chunks = []
    for n, steps in _HEAD:
        for _ in range(steps):
            chunks.append((sum(c[1] for c in chunks), n))
    HP = sum(c[1] for c in chunks)
    NU = (B * NP - HP) // _UNIT
    NR = _UNIT // _PIECE
    assert S % _PAIR == 0 and HP == NP == 1 << log_np and NP % _PIECE == 0
    assert HP + NU * _UNIT == B * NP and NU % 2 == 0 and NU >= 4 and _UNIT > 3 + NR

    def aligned(v, m):
        return v if isinstance(v, int) else pl.multiple_of(v, m)

    def kernel_function(x_hbm, w_hbm, b_ref, o_hbm, xb, ob, xh, oh, wv, bv, l_ref, e_ref, bias_ref,
                        hsem, rsem, wsem, hwsem, sem):
        def unit_piece(ref, u, r):
            q = HP + u * _UNIT + r * _PIECE
            return ref.at[q >> log_np, :, pl.ds(aligned((q & (NP - 1)) * _PAIR, _PAIR), _PIECE * _PAIR)]

        def rd_start(u):
            for r in range(NR):
                cols = pl.ds(r * _PIECE * _PAIR, _PIECE * _PAIR)
                pltpu.make_async_copy(
                    unit_piece(x_hbm, u, r), xb.at[u & 3, :, cols], rsem.at[u & 3]).start()

        def rd_wait(u):
            pltpu.make_async_copy(xb.at[u & 3], xb.at[u & 3], rsem.at[u & 3]).wait()

        def wr_start(u, r, ps=range(_PIECE)):
            dst = unit_piece(o_hbm, u, r)
            for p in ps:
                pltpu.make_async_copy(
                    ob.at[u & 3, :, pl.ds((r * _PIECE + p) * _PAIR, _PAIR)],
                    dst.at[:, pl.ds(p * _PAIR, _PAIR)], wsem.at[u & 3]).start()

        def wr_wait(u):
            pltpu.make_async_copy(ob.at[u & 3], ob.at[u & 3], wsem.at[u & 3]).wait()

        def head_rd(j, q, n):
            cols = pl.ds(aligned(q * _PAIR, _PAIR), n * _PAIR)
            return pltpu.make_async_copy(x_hbm.at[0, :, cols], xh.at[:, cols], hsem.at[j])

        def head_wr_start(r):
            for q in range(r * _PIECE, (r + 1) * _PIECE):
                cols = pl.ds(q * _PAIR, _PAIR)
                pltpu.make_async_copy(oh.at[:, cols], o_hbm.at[0, :, cols], hwsem).start()

        def pair(src, dst, q):
            cols = pl.ds(aligned(q * _PAIR, _PAIR), _PAIR)
            _compute_pair(src.at[:, cols], dst.at[:, cols], l_ref, e_ref, bias_ref)

        bcp = pltpu.make_async_copy(b_ref, bv, sem.at[len(_W_PIECES)])
        bcp.start()
        wcps = [pltpu.make_async_copy(w_hbm.at[pl.ds(r, n)], wv.at[pl.ds(r, n)], sem.at[i])
                for i, (r, n) in enumerate(_W_PIECES)]
        for cp in wcps:
            cp.start()
        bcp.wait()
        for j, (q, n) in enumerate(chunks):
            head_rd(j, q, n).start()
        bias_ref[...] = jnp.broadcast_to(bv[...].astype(f32)[None, :], (128, D)).T
        _prepare_weights(lambda i: wcps[i].wait(), wv, l_ref, e_ref)

        def head_step(j, q, n):
            head_rd(j, q, n).wait()

            @pl.when(j == 0)
            def _():
                rd_start(0)

            for c in range(n):
                pair(xh, oh, q + c)

        j0 = 0
        for n, steps in _HEAD:
            q0 = chunks[j0][0]
            if steps == 1:
                head_step(jnp.int32(j0), q0, n)
            else:
                pl.loop(0, steps)(
                    lambda j, j0=j0, q0=q0, n=n: head_step(j0 + j, q0 + j * n, n))
            j0 += steps
        rd_start(1)

        @pl.loop(0, NU)
        def _(u):
            @pl.when(u >= 4)
            def _():
                wr_wait(u - 4)

            rd_wait(u)
            odd = (u & 1) == 1
            for p in range(_UNIT):
                pair(xb.at[u & 3], ob.at[u & 3], p)
                if p == 1:
                    for k in (2, 3):
                        pl.when(~odd & (u + k < NU))(lambda k=k: rd_start(u + k))
                for i in range(2 * NR):
                    if p == 2 + i // 2:
                        back, r = 2 - i // NR, i % NR
                        pl.when(odd & (u >= back) & (u - back < NU - 3))(
                            lambda back=back, r=r: wr_start(u - back, r))
                for r in range(HP // _PIECE):
                    if p == 2 + r // 2:
                        pl.when(u == 1)(lambda r=r: head_wr_start(r))
                for r in range(NR):
                    if p == 3 + r // 2:
                        pl.when(u == NU - 2)(lambda r=r: wr_start(u - 1, r))
                pl.when(u >= NU - 2)(lambda p=p: wr_start(u, p // _PIECE, (p % _PIECE,)))

        pltpu.make_async_copy(oh, oh, hwsem).wait()
        for u in range(NU - 4, NU):
            wr_wait(u)

    xt = jnp.transpose(x, (0, 2, 1))
    ot = pl.pallas_call(
        kernel_function,
        in_specs=[pl.BlockSpec(memory_space=pl.ANY)] * 3,
        out_specs=pl.BlockSpec(memory_space=pl.ANY),
        out_shape=jax.ShapeDtypeStruct((B, D, S), x.dtype),
        scratch_shapes=[
            pltpu.VMEM((4, D, _UNIT * _PAIR), bf16),
            pltpu.VMEM((4, D, _UNIT * _PAIR), bf16),
            pltpu.VMEM((D, HP * _PAIR), bf16),
            pltpu.VMEM((D, HP * _PAIR), bf16),
            pltpu.VMEM((D, D), bf16),
            pltpu.VMEM((D,), bf16),
            pltpu.VMEM((7, _H // 2, 256), i32),
            pltpu.VMEM((3, _H // 2, 128), i32),
            pltpu.VMEM((D, 128), f32),
            pltpu.SemaphoreType.DMA((len(chunks),)),
            pltpu.SemaphoreType.DMA((4,)),
            pltpu.SemaphoreType.DMA((4,)),
            pltpu.SemaphoreType.DMA(()),
            pltpu.SemaphoreType.DMA((len(_W_PIECES) + 1,)),
        ],
        compiler_params=pltpu.CompilerParams(
            vmem_limit_bytes=80 * 1024 * 1024,
            disable_bounds_checks=True,
        ),
    )(xt, w, b)
    return jnp.transpose(ot, (0, 2, 1))
```

```python
import jax
import jax.numpy as jnp
import jax.experimental.pallas as pl
import jax.experimental.pallas.tpu as pltpu
from jax import lax

_D = 576
_H = 288
_Q = 144
_PAIR = 256
_UNIT = 20
_PIECE = 4
_PHASE = 2
_HEAD = ((2, 2), (4, 1), (8, 1))
_W_PIECES = ((512, 64), (0, 128), (256, 128), (128, 128), (384, 128))


def _prune_packed(w):
    f32, i32 = jnp.float32, jnp.int32
    R, C = w.shape
    v = pltpu.bitcast(w, i32).reshape(R // 16, 8, C)
    a0 = pltpu.bitcast((v & 0x7FFF) << 16, f32)
    a1 = pltpu.bitcast(v & 0x7FFF0000, f32)
    hi = jnp.maximum(a0, a1)
    lo = jnp.minimum(a0, a1)
    even = (lax.broadcasted_iota(i32, v.shape, 1) & 1) == 0
    hi2 = jnp.where(even, pltpu.roll(hi, 7, 1), pltpu.roll(hi, 1, 1))
    lo2 = jnp.where(even, pltpu.roll(lo, 7, 1), pltpu.roll(lo, 1, 1))
    thr = jnp.maximum(jnp.minimum(hi, hi2), jnp.maximum(lo, lo2))
    k0 = jnp.where(a0 < thr, 0, 0xFFFF)
    k1 = jnp.where(a1 < thr, 0, -65536)
    return pltpu.bitcast((v & (k0 | k1)).reshape(R // 2, C), jnp.bfloat16)


def _prepare_weights(wait, wv, l_ref, e_ref, q_ref):
    f32, bf16, i32 = jnp.float32, jnp.bfloat16, jnp.int32
    h = _H // 2
    low = lax.broadcasted_iota(i32, (h, 128), 1) < 64
    low32 = lax.broadcasted_iota(i32, (_H, 128), 1) < 64

    def piece(i):
        wait(i)
        r0, n = _W_PIECES[i]
        wp = _prune_packed(wv[r0:r0 + n])
        if n == 64:
            wp = jnp.concatenate([wp, wp], axis=0)
        v = pltpu.bitcast(wp.T, i32)
        return v[:h], v[h:]

    def mix(p, q):
        return jnp.where(low, p, q)

    def neg(p):
        return p ^ jnp.int32(-0x7FFF8000)

    def up(p):
        return pltpu.bitcast(p, bf16).astype(f32)

    def down(p):
        return pltpu.bitcast(p.astype(bf16), i32)

    top, bot = piece(0)
    first = []
    for t in range(2):
        a11, a21 = piece(1 + 2 * t)
        f11, f21 = up(a11), up(a21)
        s6 = down(f21 - f11)
        a12, a22 = piece(2 + 2 * t)
        f12, f22 = up(a12), up(a22)
        s1, s7 = down(f11 + f22), down(f12 - f22)
        if t == 0:
            tiles = (s1, a11, a22, s6, s7)
        else:
            tiles = (mix(s1, 0), mix(a11, neg(a22)), mix(a22, neg(a11)), mix(s6, bot), mix(s7, top))
            e_ref[0] = mix(pltpu.roll(s1, 64, 1), 0)
            e_ref[1] = mix(top, s7)
            e_ref[2] = mix(bot, s6)
        for i, tile in enumerate(tiles):
            l_ref[i, :, t * 128:(t + 1) * 128] = tile
        for i, g in enumerate((f21 + f22, f11 + f12)):
            if t == 0:
                g11, g21 = g[:_Q], g[_Q:]
                q_ref[i, 2] = down(g11)
                q_ref[i, 5] = down(g21 - g11)
                first.append((g11, g21))
            else:
                g = jnp.where(low32, g, -g)
                (g11, g21), g12, g22 = first[i], g[:_Q], g[_Q:]
                q_ref[i, 0] = down(g11 + g22)
                q_ref[i, 1] = down(g21 + g22)
                q_ref[i, 3] = down(g22)
                q_ref[i, 4] = down(g11 + g12)
                q_ref[i, 6] = down(g12 - g22)


def _dot(packed, t):
    return jnp.dot(pltpu.bitcast(packed, jnp.bfloat16), t.astype(jnp.bfloat16),
                   preferred_element_type=jnp.float32)


def _cat(p, q):
    return jnp.concatenate([p, q], axis=0)


def _token_operands(x_ref, c0):
    f32, bf16 = jnp.float32, jnp.bfloat16
    P, Q = pl.ds(c0, 128), pl.ds(c0 + 128, 128)
    B11, B12 = x_ref[0:256, P], x_ref[0:256, Q]
    B21, B22 = x_ref[256:512, P], x_ref[256:512, Q]
    XP, XQ = x_ref[512:, P], x_ref[512:, Q]
    f11, f12, f21, f22 = (v.astype(f32) for v in (B11, B12, B21, B22))
    zero = jnp.zeros((64, 128), bf16)
    return dict(
        M1=lambda: _cat((f11[:192] + f22[:192]).astype(bf16), zero),
        M3=lambda: f12 - f22,
        M4=lambda: f21 - f11,
        M6=lambda: _cat((f11[:192] + f12[:192]).astype(bf16), XQ),
        M7=lambda: _cat((f21[:192] + f22[:192]).astype(bf16), XP),
        N1=lambda: _cat((f12[192:] + f21[192:]).astype(bf16), zero),
        E2=lambda: _cat(XQ, (f21[192:] + f22[192:]).astype(bf16)),
        E3=lambda: _cat(XP, (f11[192:] + f12[192:]).astype(bf16)),
        M2=(_cat(B11[:192], B12[192:]), _cat(f11[:192], f12[192:])),
        M5=(_cat(B22[:192], B21[192:]), _cat(f22[:192], f21[192:])),
    )


def _compute_quad(x_ref, o_ref, l_ref, e_ref, q_ref, bias_ref):
    T = [_token_operands(x_ref, c0) for c0 in (0, _PAIR)]
    M = [{}, {}]
    for i, name in ((1, "M5"), (0, "M2")):
        (raw_a, ta), (raw_b, tb) = T[0][name], T[1][name]
        t11, t21, t12, t22 = ta[:128], ta[128:], tb[:128], tb[128:]
        m5 = _dot(q_ref[i, 4], raw_b[128:])
        m2 = _dot(q_ref[i, 1], raw_a[:128])
        m4 = _dot(q_ref[i, 3], t21 - t11)
        m3 = _dot(q_ref[i, 2], t12 - t22)
        m1 = _dot(q_ref[i, 0], t11 + t22)
        m6 = _dot(q_ref[i, 5], t11 + t12)
        m7 = _dot(q_ref[i, 6], t21 + t22)
        M[0][name] = _cat(m1 + m4 - m5 + m7, m2 + m4)
        M[1][name] = _cat(m3 + m5, m1 - m2 + m3 + m6)
    for name, ref, i in (("N1", e_ref, 0), ("M4", l_ref, 2), ("M3", l_ref, 1), ("M1", l_ref, 0),
                         ("M6", l_ref, 3), ("M7", l_ref, 4), ("E2", e_ref, 1), ("E3", e_ref, 2)):
        lhs = ref[i]
        for k in range(2):
            M[k][name] = _dot(lhs, T[k][name]())
    bf16 = jnp.bfloat16
    for m, c0 in zip(M, (0, _PAIR)):
        P, Q = pl.ds(c0, 128), pl.ds(c0 + 128, 128)
        o_ref[:_H, P] = (m["M1"] + m["M4"] - m["M5"] + m["M7"] + bias_ref[:_H]).astype(bf16)
        o_ref[:_H, Q] = (m["M3"] + m["M5"] + m["N1"] + m["E2"] + bias_ref[:_H]).astype(bf16)
        o_ref[_H:, P] = (m["M2"] + m["M4"] + m["N1"] + m["E3"] + bias_ref[_H:]).astype(bf16)
        o_ref[_H:, Q] = (m["M1"] - m["M2"] + m["M3"] + m["M6"] + bias_ref[_H:]).astype(bf16)


@jax.jit
def pallas_standalone__structured_sparse_n_m__ragged_kernel(
    x: jax.Array,
    w: jax.Array,
    b: jax.Array,
):
    f32, bf16, i32 = jnp.float32, jnp.bfloat16, jnp.int32
    B, S, D = x.shape
    assert D == _D and x.dtype == w.dtype == b.dtype == bf16
    NP = S // _PAIR
    log_np = NP.bit_length() - 1
    chunks = []
    for n, steps in _HEAD:
        for _ in range(steps):
            chunks.append((sum(c[1] for c in chunks), n))
    HP = sum(c[1] for c in chunks)
    NU = (B * NP - HP) // _UNIT
    NR = _UNIT // _PIECE
    assert S % _PAIR == 0 and HP == NP == 1 << log_np and NP % _PIECE == 0
    assert HP + NU * _UNIT == B * NP and NU % 2 == 0 and NU >= 4
    assert _UNIT % _PIECE == 0 and _PIECE % 2 == 0 and _PHASE + NR <= _UNIT // 2 and HP // _PIECE <= 2 * NR

    def aligned(v, m):
        return v if isinstance(v, int) else pl.multiple_of(v, m)

    def kernel_function(x_hbm, w_hbm, b_ref, o_hbm, xb, ob, xh, oh, wv, bv, l_ref, e_ref, q_ref,
                        bias_ref, hsem, rsem, wsem, hwsem, sem):
        def unit_piece(ref, u, r):
            q = HP + u * _UNIT + r * _PIECE
            return ref.at[q >> log_np, :, pl.ds(aligned((q & (NP - 1)) * _PAIR, _PAIR), _PIECE * _PAIR)]

        def rd_start(u, rs=range(NR)):
            for r in rs:
                cols = pl.ds(r * _PIECE * _PAIR, _PIECE * _PAIR)
                pltpu.make_async_copy(
                    unit_piece(x_hbm, u, r), xb.at[u & 3, :, cols], rsem.at[u & 3]).start()

        def rd_wait(u):
            pltpu.make_async_copy(xb.at[u & 3], xb.at[u & 3], rsem.at[u & 3]).wait()

        def wr_start(u, r, ps=range(_PIECE)):
            dst = unit_piece(o_hbm, u, r)
            for p in ps:
                pltpu.make_async_copy(
                    ob.at[u & 3, :, pl.ds((r * _PIECE + p) * _PAIR, _PAIR)],
                    dst.at[:, pl.ds(p * _PAIR, _PAIR)], wsem.at[u & 3]).start()

        def wr_wait(u):
            pltpu.make_async_copy(ob.at[u & 3], ob.at[u & 3], wsem.at[u & 3]).wait()

        def head_rd(j, q, n):
            cols = pl.ds(aligned(q * _PAIR, _PAIR), n * _PAIR)
            return pltpu.make_async_copy(x_hbm.at[0, :, cols], xh.at[:, cols], hsem.at[j])

        def head_wr_start(r):
            for q in range(r * _PIECE, (r + 1) * _PIECE):
                cols = pl.ds(q * _PAIR, _PAIR)
                pltpu.make_async_copy(oh.at[:, cols], o_hbm.at[0, :, cols], hwsem).start()

        def quad(src, dst, q):
            cols = pl.ds(aligned(q * _PAIR, 2 * _PAIR), 2 * _PAIR)
            _compute_quad(src.at[:, cols], dst.at[:, cols], l_ref, e_ref, q_ref, bias_ref)

        bcp = pltpu.make_async_copy(b_ref, bv, sem.at[len(_W_PIECES)])
        bcp.start()
        wcps = [pltpu.make_async_copy(w_hbm.at[pl.ds(r, n)], wv.at[pl.ds(r, n)], sem.at[i])
                for i, (r, n) in enumerate(_W_PIECES)]
        for cp in wcps:
            cp.start()
        bcp.wait()
        for j, (q, n) in enumerate(chunks):
            head_rd(j, q, n).start()
        bias_ref[...] = jnp.broadcast_to(bv[...].astype(f32)[None, :], (128, D)).T
        _prepare_weights(lambda i: wcps[i].wait(), wv, l_ref, e_ref, q_ref)

        def head_step(j, q, n):
            head_rd(j, q, n).wait()

            @pl.when(j == 0)
            def _():
                rd_start(0)

            for c in range(0, n, 2):
                quad(xh, oh, q + c)

        j0 = 0
        for n, steps in _HEAD:
            q0 = chunks[j0][0]
            if steps == 1:
                head_step(jnp.int32(j0), q0, n)
            else:
                pl.loop(0, steps)(
                    lambda j, j0=j0, q0=q0, n=n: head_step(j0 + j, q0 + j * n, n))
            j0 += steps
        rd_start(1)

        @pl.loop(0, NU)
        def _(u):
            @pl.when(u >= 4)
            def _():
                wr_wait(u - 4)

            rd_wait(u)
            odd = (u & 1) == 1
            for p in range(_UNIT // 2):
                quad(xb.at[u & 3], ob.at[u & 3], 2 * p)
                if _PHASE <= p < _PHASE + NR:
                    for i in (2 * (p - _PHASE), 2 * (p - _PHASE) + 1):
                        k, r = i // NR, i % NR
                        pl.when(~odd & (u + 2 + k < NU))(
                            lambda k=k, r=r: rd_start(u + 2 + k, (r,)))
                        pl.when(odd & (u >= 2 - k) & (u - 2 + k < NU - 3))(
                            lambda k=k, r=r: wr_start(u - 2 + k, r))
                    for r in (2 * (p - _PHASE), 2 * (p - _PHASE) + 1):
                        if r < HP // _PIECE:
                            pl.when(u == 1)(lambda r=r: head_wr_start(r))
                        if r < NR:
                            pl.when(u == NU - 2)(lambda r=r: wr_start(u - 1, r))
                done = (2 * p % _PIECE, 2 * p % _PIECE + 1)
                pl.when(u >= NU - 2)(lambda p=p, done=done: wr_start(u, 2 * p // _PIECE, done))

        pltpu.make_async_copy(oh, oh, hwsem).wait()
        for u in range(NU - 4, NU):
            wr_wait(u)

    xt = jnp.transpose(x, (0, 2, 1))
    ot = pl.pallas_call(
        kernel_function,
        in_specs=[pl.BlockSpec(memory_space=pl.ANY)] * 3,
        out_specs=pl.BlockSpec(memory_space=pl.ANY),
        out_shape=jax.ShapeDtypeStruct((B, D, S), x.dtype),
        scratch_shapes=[
            pltpu.VMEM((4, D, _UNIT * _PAIR), bf16),
            pltpu.VMEM((4, D, _UNIT * _PAIR), bf16),
            pltpu.VMEM((D, HP * _PAIR), bf16),
            pltpu.VMEM((D, HP * _PAIR), bf16),
            pltpu.VMEM((D, D), bf16),
            pltpu.VMEM((D,), bf16),
            pltpu.VMEM((5, _H // 2, 256), i32),
            pltpu.VMEM((3, _H // 2, 128), i32),
            pltpu.VMEM((2, 7, _Q // 2, 128), i32),
            pltpu.VMEM((D, 128), f32),
            pltpu.SemaphoreType.DMA((len(chunks),)),
            pltpu.SemaphoreType.DMA((4,)),
            pltpu.SemaphoreType.DMA((4,)),
            pltpu.SemaphoreType.DMA(()),
            pltpu.SemaphoreType.DMA((len(_W_PIECES) + 1,)),
        ],
        compiler_params=pltpu.CompilerParams(
            vmem_limit_bytes=80 * 1024 * 1024,
            disable_bounds_checks=True,
        ),
    )(xt, w, b)
    return jnp.transpose(ot, (0, 2, 1))
```

```python
import jax
import jax.numpy as jnp
import jax.experimental.pallas as pl
import jax.experimental.pallas.tpu as pltpu
from jax import lax

_D = 576
_H = 288
_Q = 144
_PAIR = 256
_UNIT = 20
_PIECE = 4
_QUAD = 512
_STEP = 3
_HEAD = ((2, 2), (4, 1), (8, 1))
_W_PIECES = ((512, 64), (0, 128), (256, 128), (128, 128), (384, 128))


def _prune_packed(w):
    f32, i32 = jnp.float32, jnp.int32
    R, C = w.shape
    v = pltpu.bitcast(w, i32).reshape(R // 16, 8, C)
    a0 = pltpu.bitcast((v & 0x7FFF) << 16, f32)
    a1 = pltpu.bitcast(v & 0x7FFF0000, f32)
    hi = jnp.maximum(a0, a1)
    lo = jnp.minimum(a0, a1)
    even = (lax.broadcasted_iota(i32, v.shape, 1) & 1) == 0
    hi2 = jnp.where(even, pltpu.roll(hi, 7, 1), pltpu.roll(hi, 1, 1))
    lo2 = jnp.where(even, pltpu.roll(lo, 7, 1), pltpu.roll(lo, 1, 1))
    thr = jnp.maximum(jnp.minimum(hi, hi2), jnp.maximum(lo, lo2))
    k0 = jnp.where(a0 < thr, 0, 0xFFFF)
    k1 = jnp.where(a1 < thr, 0, -65536)
    return pltpu.bitcast((v & (k0 | k1)).reshape(R // 2, C), jnp.bfloat16)


def _prepare_weights(wait, wv, l_ref, e_ref, q_ref):
    f32, bf16, i32 = jnp.float32, jnp.bfloat16, jnp.int32
    h = _H // 2
    low = lax.broadcasted_iota(i32, (h, 128), 1) < 64
    low32 = lax.broadcasted_iota(i32, (_H, 128), 1) < 64

    def piece(i):
        wait(i)
        r0, n = _W_PIECES[i]
        wp = _prune_packed(wv[r0:r0 + n])
        if n == 64:
            wp = jnp.concatenate([wp, wp], axis=0)
        v = pltpu.bitcast(wp.T, i32)
        return v[:h], v[h:]

    def mix(p, q):
        return jnp.where(low, p, q)

    def neg(p):
        return p ^ jnp.int32(-0x7FFF8000)

    def up(p):
        return pltpu.bitcast(p, bf16).astype(f32)

    def down(p):
        return pltpu.bitcast(p.astype(bf16), i32)

    top, bot = piece(0)
    first = []
    for t in range(2):
        a11, a21 = piece(1 + 2 * t)
        f11, f21 = up(a11), up(a21)
        s6 = down(f21 - f11)
        a12, a22 = piece(2 + 2 * t)
        f12, f22 = up(a12), up(a22)
        s1, s7 = down(f11 + f22), down(f12 - f22)
        if t == 0:
            tiles = (s1, a11, a22, s6, s7)
        else:
            tiles = (mix(s1, 0), mix(a11, neg(a22)), mix(a22, neg(a11)), mix(s6, bot), mix(s7, top))
            e_ref[0] = mix(pltpu.roll(s1, 64, 1), 0)
            e_ref[1] = mix(top, s7)
            e_ref[2] = mix(bot, s6)
        for i, tile in enumerate(tiles):
            l_ref[i, :, t * 128:(t + 1) * 128] = tile
        for i, g in enumerate((f21 + f22, f11 + f12)):
            if t == 0:
                g11, g21 = g[:_Q], g[_Q:]
                q_ref[i, 2] = down(g11)
                q_ref[i, 5] = down(g21 - g11)
                first.append((g11, g21))
            else:
                g = jnp.where(low32, g, -g)
                (g11, g21), g12, g22 = first[i], g[:_Q], g[_Q:]
                q_ref[i, 0] = down(g11 + g22)
                q_ref[i, 1] = down(g21 + g22)
                q_ref[i, 3] = down(g22)
                q_ref[i, 4] = down(g11 + g12)
                q_ref[i, 6] = down(g12 - g22)


def _dot(packed, t):
    return jnp.dot(pltpu.bitcast(packed, jnp.bfloat16), t.astype(jnp.bfloat16),
                   preferred_element_type=jnp.float32)


def _cat(p, q):
    return jnp.concatenate([p, q], axis=0)


def _token_operands(x_ref, c0):
    f32, bf16 = jnp.float32, jnp.bfloat16
    P, Q = pl.ds(c0, 128), pl.ds(c0 + 128, 128)
    B11, B12 = x_ref[0:256, P], x_ref[0:256, Q]
    B21, B22 = x_ref[256:512, P], x_ref[256:512, Q]
    XP, XQ = x_ref[512:, P], x_ref[512:, Q]
    f11, f12, f21, f22 = (v.astype(f32) for v in (B11, B12, B21, B22))
    zero = jnp.zeros((64, 128), bf16)
    return dict(
        M1=lambda: _cat((f11[:192] + f22[:192]).astype(bf16), zero),
        M3=lambda: f12 - f22,
        M4=lambda: f21 - f11,
        M6=lambda: _cat((f11[:192] + f12[:192]).astype(bf16), XQ),
        M7=lambda: _cat((f21[:192] + f22[:192]).astype(bf16), XP),
        N1=lambda: _cat((f12[192:] + f21[192:]).astype(bf16), zero),
        E2=lambda: _cat(XQ, (f21[192:] + f22[192:]).astype(bf16)),
        E3=lambda: _cat(XP, (f11[192:] + f12[192:]).astype(bf16)),
        M2=_cat(f11[:192], f12[192:]),
        M5=_cat(f22[:192], f21[192:]),
    )


def _compute_quad(x_ref, o_ref, l_ref, e_ref, q_ref, bias_ref, between=None):
    m = {}
    m[1, 2] = _dot(q_ref[1, 1], x_ref[256:384, 128:256])
    m[0, 2] = _dot(q_ref[0, 1], x_ref[0:128, 0:128])
    m[1, 5] = _dot(q_ref[1, 4], _cat(x_ref[384:448, 384:512], x_ref[448:512, 256:384]))
    m[0, 5] = _dot(q_ref[0, 4], _cat(x_ref[128:192, 256:384], x_ref[192:256, 384:512]))
    T = [_token_operands(x_ref, c0) for c0 in (0, _PAIR)]
    M = [{}, {}]
    for i, name in ((1, "M5"), (0, "M2")):
        ta, tb = T[0][name], T[1][name]
        t11, t21, t12, t22 = ta[:128], ta[128:], tb[:128], tb[128:]
        m5, m2 = m[i, 5], m[i, 2]
        m4 = _dot(q_ref[i, 3], t21 - t11)
        m3 = _dot(q_ref[i, 2], t12 - t22)
        m1 = _dot(q_ref[i, 0], t11 + t22)
        m6 = _dot(q_ref[i, 5], t11 + t12)
        m7 = _dot(q_ref[i, 6], t21 + t22)
        M[0][name] = _cat(m1 + m4 - m5 + m7, m2 + m4)
        M[1][name] = _cat(m3 + m5, m1 - m2 + m3 + m6)
    plain = (("M4", l_ref, 2), ("M1", l_ref, 0), ("M3", l_ref, 1), ("N1", e_ref, 0),
             ("M7", l_ref, 4), ("M6", l_ref, 3), ("E3", e_ref, 2), ("E2", e_ref, 1))

    def store(k):
        m, bf16 = M[k], jnp.bfloat16
        P, Q = pl.ds(k * _PAIR, 128), pl.ds(k * _PAIR + 128, 128)
        o_ref[:_H, P] = (m["M1"] + m["M4"] - m["M5"] + m["M7"] + bias_ref[:_H]).astype(bf16)
        o_ref[:_H, Q] = (m["M3"] + m["M5"] + m["N1"] + m["E2"] + bias_ref[:_H]).astype(bf16)
        o_ref[_H:, P] = (m["M2"] + m["M4"] + m["N1"] + m["E3"] + bias_ref[_H:]).astype(bf16)
        o_ref[_H:, Q] = (m["M1"] - m["M2"] + m["M3"] + m["M6"] + bias_ref[_H:]).astype(bf16)

    if between is None:
        for name, ref, i in plain:
            for k in range(2):
                M[k][name] = _dot(ref[i], T[k][name]())
        store(0)
        store(1)
    else:
        for k in range(2):
            for name, ref, i in plain:
                M[k][name] = _dot(ref[i], T[k][name]())
            store(k)
            between(k)


@jax.jit
def pallas_standalone__structured_sparse_n_m__ragged_kernel(
    x: jax.Array,
    w: jax.Array,
    b: jax.Array,
):
    f32, bf16, i32 = jnp.float32, jnp.bfloat16, jnp.int32
    B, S, D = x.shape
    assert D == _D and x.dtype == w.dtype == b.dtype == bf16
    NP = S // _PAIR
    log_np = NP.bit_length() - 1
    chunks = []
    for n, steps in _HEAD:
        for _ in range(steps):
            chunks.append((sum(c[1] for c in chunks), n))
    HP = sum(c[1] for c in chunks)
    NU = (B * NP - HP) // _UNIT
    NR = _UNIT // _PIECE
    assert S % _PAIR == 0 and HP == NP == 1 << log_np and NP % _PIECE == 0
    assert HP + NU * _UNIT == B * NP and NU % 2 == 0 and NU >= 4
    assert _UNIT % _PIECE == 0 and _PIECE % 2 == 0 and _STEP + NR <= _UNIT // 2 and HP // _PIECE <= 2 * NR

    def aligned(v, m):
        return v if isinstance(v, int) else pl.multiple_of(v, m)

    def kernel_function(x_hbm, w_hbm, b_ref, o_hbm, xb, ob, xh, oh, wv, bv, l_ref, e_ref, q_ref,
                        bias_ref, hsem, rsem, wsem, hwsem, sem):
        def unit_piece(ref, u, r):
            q = HP + u * _UNIT + r * _PIECE
            return ref.at[q >> log_np, :, pl.ds(aligned((q & (NP - 1)) * _PAIR, _PAIR), _PIECE * _PAIR)]

        def rd_first(u):
            for r in range(NR):
                cols = pl.ds(r * _PIECE * _PAIR, _PIECE * _PAIR)
                pltpu.make_async_copy(
                    unit_piece(x_hbm, u, r), xb.at[u & 3, :, cols], rsem.at[u & 3]).start()

        def rd_start(u, r):
            src = unit_piece(x_hbm, u, r)
            for i in range(_PIECE * _PAIR // _QUAD):
                pltpu.make_async_copy(
                    src.at[:, pl.ds(i * _QUAD, _QUAD)],
                    xb.at[u & 3, :, pl.ds(r * _PIECE * _PAIR + i * _QUAD, _QUAD)],
                    rsem.at[u & 3]).start(priority=i % 2)

        def rd_wait(u):
            pltpu.make_async_copy(xb.at[u & 3], xb.at[u & 3], rsem.at[u & 3]).wait()

        def wr_start(u, r, ps=range(_PIECE)):
            dst = unit_piece(o_hbm, u, r)
            for p in ps:
                pltpu.make_async_copy(
                    ob.at[u & 3, :, pl.ds((r * _PIECE + p) * _PAIR, _PAIR)],
                    dst.at[:, pl.ds(p * _PAIR, _PAIR)], wsem.at[u & 3]).start()

        def wr_wait(u):
            pltpu.make_async_copy(ob.at[u & 3], ob.at[u & 3], wsem.at[u & 3]).wait()

        def head_rd(j, q, n):
            cols = pl.ds(aligned(q * _PAIR, _PAIR), n * _PAIR)
            return pltpu.make_async_copy(x_hbm.at[0, :, cols], xh.at[:, cols], hsem.at[j])

        def head_wr_start(r):
            for q in range(r * _PIECE, (r + 1) * _PIECE):
                cols = pl.ds(q * _PAIR, _PAIR)
                pltpu.make_async_copy(oh.at[:, cols], o_hbm.at[0, :, cols], hwsem).start()

        def quad(src, dst, q, between=None):
            cols = pl.ds(aligned(q * _PAIR, _QUAD), _QUAD)
            _compute_quad(src.at[:, cols], dst.at[:, cols], l_ref, e_ref, q_ref, bias_ref, between)

        bcp = pltpu.make_async_copy(b_ref, bv, sem.at[len(_W_PIECES)])
        bcp.start()
        wcps = [pltpu.make_async_copy(w_hbm.at[pl.ds(r, n)], wv.at[pl.ds(r, n)], sem.at[i])
                for i, (r, n) in enumerate(_W_PIECES)]
        for cp in wcps:
            cp.start()
        bcp.wait()
        for j, (q, n) in enumerate(chunks):
            head_rd(j, q, n).start()
        bias_ref[...] = jnp.broadcast_to(bv[...].astype(f32)[None, :], (128, D)).T
        _prepare_weights(lambda i: wcps[i].wait(), wv, l_ref, e_ref, q_ref)

        def head_step(j, q, n):
            head_rd(j, q, n).wait()

            @pl.when(j == 0)
            def _():
                rd_first(0)

            for c in range(0, n, 2):
                quad(xh, oh, q + c)

        j0 = 0
        for n, steps in _HEAD:
            q0 = chunks[j0][0]
            if steps == 1:
                head_step(jnp.int32(j0), q0, n)
            else:
                pl.loop(0, steps)(
                    lambda j, j0=j0, q0=q0, n=n: head_step(j0 + j, q0 + j * n, n))
            j0 += steps
        rd_first(1)


        @pl.loop(0, NU)
        def _(u):
            @pl.when(u >= 4)
            def _():
                wr_wait(u - 4)

            rd_wait(u)
            odd = (u & 1) == 1
            for p in range(_UNIT // 2):
                r0, p0 = divmod(2 * p, _PIECE)
                if p < _UNIT // 2 - 1:
                    quad(xb.at[u & 3], ob.at[u & 3], 2 * p)
                    pl.when(u >= NU - 2)(lambda: wr_start(u, r0, (p0, p0 + 1)))
                else:
                    quad(xb.at[u & 3], ob.at[u & 3], 2 * p, lambda k: pl.when(u >= NU - 2)(
                        lambda: wr_start(u, r0, (p0 + k,))))
                if _STEP <= p < _STEP + NR:
                    for i in (2 * (p - _STEP), 2 * (p - _STEP) + 1):
                        k, r = i // NR, i % NR
                        pl.when(~odd & (u + 2 + k < NU))(
                            lambda k=k, r=r: rd_start(u + 2 + k, r))
                        pl.when(odd & (u >= 2 - k) & (u - 2 + k < NU - 3))(
                            lambda k=k, r=r: wr_start(u - 2 + k, r))
                    for r in (2 * (p - _STEP), 2 * (p - _STEP) + 1):
                        if r < HP // _PIECE:
                            pl.when(u == 1)(lambda r=r: head_wr_start(r))
                        if r < NR:
                            pl.when(u == NU - 2)(lambda r=r: wr_start(u - 1, r))

        pltpu.make_async_copy(oh, oh, hwsem).wait()
        for u in range(NU - 4, NU):
            wr_wait(u)

    xt = jnp.transpose(x, (0, 2, 1))
    ot = pl.pallas_call(
        kernel_function,
        in_specs=[pl.BlockSpec(memory_space=pl.ANY)] * 3,
        out_specs=pl.BlockSpec(memory_space=pl.ANY),
        out_shape=jax.ShapeDtypeStruct((B, D, S), x.dtype),
        scratch_shapes=[
            pltpu.VMEM((4, D, _UNIT * _PAIR), bf16),
            pltpu.VMEM((4, D, _UNIT * _PAIR), bf16),
            pltpu.VMEM((D, HP * _PAIR), bf16),
            pltpu.VMEM((D, HP * _PAIR), bf16),
            pltpu.VMEM((D, D), bf16),
            pltpu.VMEM((D,), bf16),
            pltpu.VMEM((5, _H // 2, 256), i32),
            pltpu.VMEM((3, _H // 2, 128), i32),
            pltpu.VMEM((2, 7, _Q // 2, 128), i32),
            pltpu.VMEM((D, 128), f32),
            pltpu.SemaphoreType.DMA((len(chunks),)),
            pltpu.SemaphoreType.DMA((4,)),
            pltpu.SemaphoreType.DMA((4,)),
            pltpu.SemaphoreType.DMA(()),
            pltpu.SemaphoreType.DMA((len(_W_PIECES) + 1,)),
        ],
        compiler_params=pltpu.CompilerParams(
            vmem_limit_bytes=80 * 1024 * 1024,
            disable_bounds_checks=True,
        ),
    )(xt, w, b)
    return jnp.transpose(ot, (0, 2, 1))
```
